```python
import jax
import jax.numpy as jnp

def _softmax(x, axis=-1):
    return jax.nn.softmax(x, axis=axis)
def _gelu(x):
    return jax.nn.gelu(x, approximate=True)
def _silu(x):
    return jax.nn.silu(x)
def _sigmoid(x):
    return jax.nn.sigmoid(x)
def _layernorm(x, axis=-1, eps=1e-5):
    m = jnp.mean(x, axis=axis, keepdims=True)
    v = jnp.var(x, axis=axis, keepdims=True)
    return (x - m) / jnp.sqrt(v + eps)
def _scatter_add(tgt, idx, src, axis=0):
    return tgt.at[idx].add(src)
def _segment_sum(src, seg, n):
    return jax.ops.segment_sum(src, seg, n)
class _Rng:
    def __init__(self, key):
        self._k = key
    def _next(self):
        self._k, sub = jax.random.split(self._k)
        return sub
    def normal(self, shape):
        return jax.random.normal(self._next(), shape, dtype=jnp.bfloat16)
    def randint(self, lo, hi, shape):
        return jax.random.randint(self._next(), shape, lo, hi, dtype=jnp.int32)
    def uniform(self, shape, lo=0.0, hi=1.0):
        return jax.random.uniform(self._next(), shape, jnp.bfloat16, lo, hi)
    def permutation(self, n):
        return jax.random.permutation(self._next(), n)


kernel_name = 'concat_heads__spectral_gfnet__compressed_kv_cla__prompt'

def setup_inputs():
    _rng = _Rng(jax.random.key(int.from_bytes(__import__("os").urandom(4), "little")))
    _w = (lambda a: (lambda t: t.astype(jnp.bfloat16) if jnp.issubdtype(t.dtype, jnp.floating) else t)(jnp.asarray(a)))
    def _A_setup():
        B, S, D = 1, 2048, 448
        Df = D // 2 + 1
        return {
            "x": _w((lambda *s: _rng.normal(s) * 0.05)(B, S, D)),
            "w_r": _w((lambda *s: _rng.normal(s) * 0.05)(S, Df) * 0.02),
            "w_i": _w((lambda *s: _rng.normal(s) * 0.05)(S, Df) * 0.02),
        }
    _A_in = _A_setup()

    def _B_setup():
        B, H, Sq, Sk, D, M = 1, 16, 2048, 2048, 256, 448
        Dc = 4 * D
        return {
            "x": _w((lambda *s: _rng.normal(s) * 0.05)(B, Sq, M)),
            "c_kv": _w((lambda *s: _rng.normal(s) * 0.05)(B, Sk, Dc)),
            "w_q": _w((lambda *s: _rng.normal(s) * 0.05)(M, H, D) * (M ** -0.5)),
            "w_uk": _w((lambda *s: _rng.normal(s) * 0.05)(Dc, H, D) * (Dc ** -0.5)),
            "w_uv": _w((lambda *s: _rng.normal(s) * 0.05)(Dc, H, D) * (Dc ** -0.5)),
            "w_o": _w((lambda *s: _rng.normal(s) * 0.05)(H, D, M) * ((H * D) ** -0.5)),
        }
    _B_in = _B_setup()

    return {
        "A_x": _A_in["x"],
        "A_w_r": _A_in["w_r"],
        "A_w_i": _A_in["w_i"],
        "B_x": _B_in["x"],
        "B_c_kv": _B_in["c_kv"],
        "B_w_q": _B_in["w_q"],
        "B_w_uk": _B_in["w_uk"],
        "B_w_uv": _B_in["w_uv"],
        "B_w_o": _B_in["w_o"],
    }

def reference(A_x, A_w_r, A_w_i, B_x, B_c_kv, B_w_q, B_w_uk, B_w_uv, B_w_o):
    def _A_ref(x, w_r, w_i):
        B, S, D = x.shape
        X = (lambda x, axes=(-2,-1): jnp.fft.rfft2(x.astype(jnp.float32), axes=axes))(x, axes=(-2, -1))
        W = w_r + 1j * w_i
        X = X * W
        y = (lambda x, s, axes=(-2,-1): jnp.fft.irfft2(x, s=s, axes=axes).astype(jnp.bfloat16))(X, (S, D), axes=(-2, -1))
        return y

    def _B_ref(x, c_kv, w_q, w_uk, w_uv, w_o):
        B, Sq, M = x.shape[0], x.shape[1], x.shape[2]
        Sk = c_kv.shape[1]
        H, D = w_q.shape[1], w_q.shape[2]
        q = jnp.einsum("bqm,mhd->bhqd", x, w_q)
        k = jnp.einsum("bkc,chd->bhkd", c_kv, w_uk)
        v = jnp.einsum("bkc,chd->bhkd", c_kv, w_uv)
        scores = jnp.einsum("bhqd,bhkd->bhqk", q, k) * (D ** -0.5)
        off = Sk - Sq
        qi = jnp.arange(Sq)[:, None]
        kj = jnp.arange(Sk)[None, :]
        cmask = kj <= (qi + off)
        scores = jnp.where(cmask[None, None], scores, -1e9)
        p = _softmax(scores, axis=-1)
        ctx = jnp.einsum("bhqk,bhkd->bhqd", p, v)
        return jnp.einsum("bhqd,hdm->bqm", ctx, w_o)

    a = _A_ref(A_x, A_w_r, A_w_i)
    b = _B_ref(B_x, B_c_kv, B_w_q, B_w_uk, B_w_uv, B_w_o)
    return jnp.concatenate([a, b], axis=-1)
```

```python
import math

import jax
import jax.numpy as jnp
import ml_dtypes
import numpy as np
import jax.experimental.pallas as pl
import jax.experimental.pallas.tpu as pltpu

S, M, H, D, DC = 2048, 448, 16, 256, 1024
NF = M // 2 + 1
R = 8
S2 = S // R
TQ = 256
BF = ml_dtypes.bfloat16


def _consts():
    d = np.arange(M, dtype=np.float64)
    k = np.arange(256, dtype=np.float64)
    ang = 2 * np.pi * ((d[:, None] * k[None, :]) % M) / M
    valid = (k < NF)[None, :]
    fwd = np.concatenate([np.cos(ang) * valid, -np.sin(ang) * valid], axis=1)
    wt = np.where((k == 0) | (k == M // 2), 1.0, 2.0)[None, :] * valid
    inv = np.concatenate([(np.cos(ang) * wt).T, (-np.sin(ang) * wt).T], axis=0)
    k2 = np.arange(S2)
    mats = []
    for k1 in range(R):
        a = 2 * np.pi * (((k1 + R * k2)[:, None] * k2[None, :]) % S) / S
        mats.append(np.concatenate([np.cos(a), np.sin(a)], axis=0))
    return fwd.astype(BF), inv.astype(BF), np.stack(mats).astype(BF)


_FWD, _INV, _MS = _consts()


def _fft(xs, sign):
    n = len(xs)
    if n == 1:
        return xs
    ev, od = _fft(xs[0::2], sign), _fft(xs[1::2], sign)
    out = [None] * n
    for k in range(n // 2):
        er, ei = ev[k]
        orr, oi = od[k]
        if k == 0:
            tr, ti = orr, oi
        elif 4 * k == n:
            tr, ti = (oi, -orr) if sign < 0 else (-oi, orr)
            if sign < 0:
                out[k] = (er + oi, ei - orr)
                out[k + n // 2] = (er - oi, ei + orr)
            else:
                out[k] = (er - oi, ei + orr)
                out[k + n // 2] = (er + oi, ei - orr)
            continue
        else:
            c = math.cos(2 * math.pi * k / n)
            s = sign * math.sin(2 * math.pi * k / n)
            tr, ti = orr * c - oi * s, orr * s + oi * c
        out[k] = (er + tr, ei + ti)
        out[k + n // 2] = (er - tr, ei - ti)
    return out


def _kernel(ax_ref, wr_ref, wi_ref, fwd_ref, inv_ref, ms_ref,
            x_ref, c_ref, wq_ref, wuk_ref, wuv_ref, wo_ref,
            o_ref,
            q_s, k_s, v_s, acc_s, z_s, b_s, w_s):
    step = pl.program_id(0)
    f32, bf16 = jnp.float32, jnp.bfloat16

    @pl.when(step == 0)
    def _init():
        acc_s[...] = jnp.zeros_like(acc_s)

    @pl.when(step < H)
    def _head():
        qscale = (D ** -0.5) * math.log2(math.e)
        for r in range(0, S, 512):
            q = jnp.dot(x_ref[0, r:r + 512, :], wq_ref[...], preferred_element_type=f32)
            q_s[r:r + 512, :] = (q * qscale).astype(bf16)
            c = c_ref[0, r:r + 512, :]
            k_s[r:r + 512, :] = jnp.dot(c, wuk_ref[...], preferred_element_type=f32).astype(bf16)
            v_s[r:r + 512, :] = jnp.dot(c, wuv_ref[...], preferred_element_type=f32).astype(bf16)
        nt = (((1,), (1,)), ((), ()))
        tri = (jax.lax.broadcasted_iota(jnp.int32, (TQ, TQ), 1)
               <= jax.lax.broadcasted_iota(jnp.int32, (TQ, TQ), 0))
        for i in range(S // TQ):
            r0 = i * TQ
            q = q_s[r0:r0 + TQ, :]
            sd = jax.lax.dot_general(q, k_s[r0:r0 + TQ, :], nt, preferred_element_type=f32)
            sd = jnp.where(tri, sd, -1e30)
            m = jnp.max(sd, axis=1, keepdims=True)
            if i:
                so = jax.lax.dot_general(q, k_s[0:r0, :], nt, preferred_element_type=f32)
                m = jnp.maximum(m, jnp.max(so, axis=1, keepdims=True))
            pd = jnp.exp2(sd - m)
            l = jnp.sum(pd, axis=1, keepdims=True)
            ctx = jnp.dot(pd.astype(bf16), v_s[r0:r0 + TQ, :], preferred_element_type=f32)
            if i:
                po = jnp.exp2(so - m)
                l = l + jnp.sum(po, axis=1, keepdims=True)
                ctx = ctx + jnp.dot(po.astype(bf16), v_s[0:r0, :], preferred_element_type=f32)
            ctx = (ctx * (1.0 / l)).astype(bf16)
            acc_s[r0:r0 + TQ, :] += jnp.dot(ctx, wo_ref[0], preferred_element_type=f32)

    @pl.when(step == H - 1)
    def _emit():
        for r in range(0, S, 256):
            o_ref[0, r:r + 256, M:2 * M] = acc_s[r:r + 256, :].astype(bf16)

    @pl.when(step == H)
    def _spectral():
        for j, w_ref in enumerate((wr_ref, wi_ref)):
            w_s[2 * j + 1] = jnp.zeros((S, 128), f32)
            for r in range(0, S, 256):
                w_s[2 * j, r:r + 256, :] = w_ref[r:r + 256, 0:128].astype(f32)
                w_s[2 * j + 1, r:r + 256, 0:NF - 128] = w_ref[r:r + 256, 128:NF].astype(f32)
        for r in range(0, S, 256):
            z_s[r:r + 256, :] = jnp.dot(ax_ref[0, r:r + 256, :], fwd_ref[...],
                                        preferred_element_type=f32)

        def butterfly(sign):
            def body(t, carry):
                r = pl.multiple_of(t * 16, 16)
                xs = [(z_s[pl.ds(n * S2 + r, 16), 0:256], z_s[pl.ds(n * S2 + r, 16), 256:512])
                      for n in range(R)]
                ys = _fft(xs, sign)
                for n in range(R):
                    b_s[pl.ds(n * S2 + r, 16), 0:256] = ys[n][0].astype(bf16)
                    b_s[pl.ds(n * S2 + r, 16), 256:512] = ys[n][1].astype(bf16)
                return carry
            jax.lax.fori_loop(0, S2 // 16, body, 0)

        butterfly(-1)
        for k1 in range(R):
            t = jnp.dot(ms_ref[k1], b_s[k1 * S2:(k1 + 1) * S2, :], preferred_element_type=f32)
            gr = t[0:256, 0:256] + t[256:512, 256:512]
            gi = t[0:256, 256:512] - t[256:512, 0:256]
            rows = pl.ds(k1, S2, stride=R)
            wr = jnp.concatenate([w_s[0, rows, :], w_s[1, rows, :]], axis=1)
            wi = jnp.concatenate([w_s[2, rows, :], w_s[3, rows, :]], axis=1)
            yr = (gr * wr - gi * wi).astype(bf16)
            yi = (gr * wi + gi * wr).astype(bf16)
            rhs = jnp.concatenate([jnp.concatenate([yr, yi], axis=1),
                                   jnp.concatenate([-yi, yr], axis=1)], axis=0)
            z_s[k1 * S2:(k1 + 1) * S2, :] = jax.lax.dot_general(
                ms_ref[k1], rhs, (((0,), (0,)), ((), ())), preferred_element_type=f32)
        butterfly(+1)
        for r in range(0, S, 256):
            y = jnp.dot(b_s[r:r + 256, :], inv_ref[...], preferred_element_type=f32)
            o_ref[0, r:r + 256, 0:M] = (y * (1.0 / (S * M))).astype(bf16)


@jax.jit
def pallas_concat_heads__spectral_gfnet__compressed_kv_cla__prompt_kernel(
    A_x, A_w_r, A_w_i, B_x, B_c_kv, B_w_q, B_w_uk, B_w_uv, B_w_o,
):
    def full(shape):
        n = len(shape)
        return pl.BlockSpec(shape, lambda h: (0,) * n, pipeline_mode=pl.Buffered(1))

    def head(rows):
        return pl.BlockSpec((rows, D), lambda h: (0, jnp.minimum(h, H - 1)))

    return pl.pallas_call(
        _kernel,
        grid=(H + 1,),
        in_specs=[
            full((1, S, M)), full((S, NF)), full((S, NF)),
            full(_FWD.shape), full(_INV.shape), full(_MS.shape),
            full((1, S, M)), full((1, S, DC)),
            head(M), head(DC), head(DC),
            pl.BlockSpec((1, D, M), lambda h: (jnp.minimum(h, H - 1), 0, 0)),
        ],
        out_specs=pl.BlockSpec((1, S, 2 * M), lambda h: (0, 0, 0)),
        out_shape=jax.ShapeDtypeStruct((1, S, 2 * M), jnp.bfloat16),
        scratch_shapes=[
            pltpu.VMEM((S, D), jnp.bfloat16), pltpu.VMEM((S, D), jnp.bfloat16),
            pltpu.VMEM((S, D), jnp.bfloat16), pltpu.VMEM((S, M), jnp.float32),
            pltpu.VMEM((S, 512), jnp.float32), pltpu.VMEM((S, 512), jnp.bfloat16),
            pltpu.VMEM((4, S, 128), jnp.float32),
        ],
        compiler_params=pltpu.CompilerParams(
            dimension_semantics=("arbitrary",), vmem_limit_bytes=100 * 1024 * 1024),
    )(A_x, A_w_r, A_w_i, _FWD, _INV, _MS,
      B_x, B_c_kv, B_w_q.reshape(M, H * D), B_w_uk.reshape(DC, H * D),
      B_w_uv.reshape(DC, H * D), B_w_o)
```

```python
import math

import jax
import jax.numpy as jnp
import ml_dtypes
import numpy as np
import jax.experimental.pallas as pl
import jax.experimental.pallas.tpu as pltpu

S, M, H, D, DC = 2048, 448, 16, 256, 1024
NF = M // 2 + 1
R = 8
S2 = S // R
TQ = 256
BF = ml_dtypes.bfloat16


def _consts():
    d = np.arange(M, dtype=np.float64)
    k = np.arange(256, dtype=np.float64)
    ang = 2 * np.pi * ((d[:, None] * k[None, :]) % M) / M
    valid = (k < NF)[None, :]
    fwd = np.concatenate([np.cos(ang) * valid, -np.sin(ang) * valid], axis=1)
    wt = np.where((k == 0) | (k == M // 2), 1.0, 2.0)[None, :] * valid
    inv = np.concatenate([(np.cos(ang) * wt).T, (-np.sin(ang) * wt).T], axis=0)
    k2 = np.arange(S2)
    mats = []
    for k1 in range(R):
        a = 2 * np.pi * (((k1 + R * k2)[:, None] * k2[None, :]) % S) / S
        mats.append(np.concatenate([np.cos(a), np.sin(a)], axis=0))
    return fwd.astype(BF), inv.astype(BF), np.stack(mats).astype(BF)


_FWD, _INV, _MS = _consts()


def _fft(xs, sign):
    n = len(xs)
    if n == 1:
        return xs
    ev, od = _fft(xs[0::2], sign), _fft(xs[1::2], sign)
    out = [None] * n
    for k in range(n // 2):
        er, ei = ev[k]
        orr, oi = od[k]
        if k == 0:
            tr, ti = orr, oi
        elif 4 * k == n:
            tr, ti = (oi, -orr) if sign < 0 else (-oi, orr)
            if sign < 0:
                out[k] = (er + oi, ei - orr)
                out[k + n // 2] = (er - oi, ei + orr)
            else:
                out[k] = (er - oi, ei + orr)
                out[k + n // 2] = (er + oi, ei - orr)
            continue
        else:
            c = math.cos(2 * math.pi * k / n)
            s = sign * math.sin(2 * math.pi * k / n)
            tr, ti = orr * c - oi * s, orr * s + oi * c
        out[k] = (er + tr, ei + ti)
        out[k + n // 2] = (er - tr, ei - ti)
    return out


def _kernel(ax_ref, wr_ref, wi_ref, fwd_ref, inv_ref, ms_ref,
            xt_ref, c_hbm, wq_hbm, wuk_hbm, wuv_hbm, wo_hbm,
            o_ref,
            q_s, k_s, v_s, acc_s, z_s, b_s, w_s, xs_s,
            c_ref, rq_s, rk_s, rv_s, wq_s, wuk_s, wuv_s, wo_ref, sems):
    step = pl.program_id(0)
    f32, bf16 = jnp.float32, jnp.bfloat16

    copies = [pltpu.make_async_copy(a, b, sems.at[i]) for i, (a, b) in enumerate(
        ((wq_hbm, rq_s), (c_hbm, c_ref), (wuk_hbm, rk_s), (wuv_hbm, rv_s), (wo_hbm, wo_ref)))]

    @pl.when(step == 0)
    def _start():
        for cp in copies:
            cp.start()

    @pl.when(step == 1)
    def _init():
        acc_s[...] = jnp.zeros_like(acc_s)
        for r in range(0, S, 256):
            xs_s[r:r + 256, :] = xt_ref[:, r:r + 256].astype(f32).T.astype(bf16)

        def relayout(src, dst, n):
            def body(t, carry):
                r = pl.multiple_of(t * 64, 64)
                dst[:, pl.ds(r, 64), :] = jnp.swapaxes(src[pl.ds(r, 64)], 0, 1)
                return carry
            jax.lax.fori_loop(0, n // 64, body, 0)
        copies[0].wait()
        relayout(rq_s, wq_s, M)
        copies[1].wait()
        copies[2].wait()
        relayout(rk_s, wuk_s, DC)
        copies[3].wait()
        relayout(rv_s, wuv_s, DC)
        copies[4].wait()

    @pl.when(step > 0)
    def _head():
        h = step - 1
        wq_ref, wuk_ref, wuv_ref = wq_s.at[h], wuk_s.at[h], wuv_s.at[h]
        qscale = (D ** -0.5) * math.log2(math.e)
        for r in range(0, S, 512):
            q = jnp.dot(xs_s[r:r + 512, :], wq_ref[...], preferred_element_type=f32)
            q_s[r:r + 512, :] = (q * qscale).astype(bf16)
            c = c_ref[r:r + 512, :]
            k_s[r:r + 512, :] = jnp.dot(c, wuk_ref[...], preferred_element_type=f32).astype(bf16)
            v_s[r:r + 512, :] = jnp.dot(c, wuv_ref[...], preferred_element_type=f32).astype(bf16)
        nt = (((1,), (1,)), ((), ()))
        tri = (jax.lax.broadcasted_iota(jnp.int32, (TQ, TQ), 1)
               <= jax.lax.broadcasted_iota(jnp.int32, (TQ, TQ), 0))
        for i in range(S // TQ):
            r0 = i * TQ
            q = q_s[r0:r0 + TQ, :]
            sd = jax.lax.dot_general(q, k_s[r0:r0 + TQ, :], nt, preferred_element_type=f32)
            sd = jnp.where(tri, sd, -1e30)
            m = jnp.max(sd, axis=1, keepdims=True)
            if i:
                so = jax.lax.dot_general(q, k_s[0:r0, :], nt, preferred_element_type=f32)
                m = jnp.maximum(m, jnp.max(so, axis=1, keepdims=True))
            pd = jnp.exp2(sd - m)
            l = jnp.sum(pd, axis=1, keepdims=True)
            ctx = jnp.dot(pd.astype(bf16), v_s[r0:r0 + TQ, :], preferred_element_type=f32)
            if i:
                po = jnp.exp2(so - m)
                l = l + jnp.sum(po, axis=1, keepdims=True)
                ctx = ctx + jnp.dot(po.astype(bf16), v_s[0:r0, :], preferred_element_type=f32)
            ctx = (ctx * (1.0 / l)).astype(bf16)
            acc_s[r0:r0 + TQ, :] += jax.lax.dot_general(ctx, wo_ref[h], nt, preferred_element_type=f32)

    @pl.when(step == H)
    def _emit():
        for r in range(0, S, 256):
            o_ref[0, r:r + 256, M:2 * M] = acc_s[r:r + 256, :].astype(bf16)

    @pl.when(step == 0)
    def _spectral():
        for j, w_ref in enumerate((wr_ref, wi_ref)):
            for r in range(0, S, 256):
                w_s[2 * j, r:r + 256, :] = w_ref[0:128, r:r + 256].astype(f32).T
                hi = jnp.concatenate([w_ref[128:224, r:r + 256].astype(f32),
                                      jnp.broadcast_to(w_ref[224:225, r:r + 256].astype(f32), (32, 256))],
                                     axis=0)
                hi = jnp.where(jax.lax.broadcasted_iota(jnp.int32, (128, 256), 0) < NF - 128, hi, 0.0)
                w_s[2 * j + 1, r:r + 256, :] = hi.T
        for r in range(0, S, 256):
            z_s[r:r + 256, :] = jax.lax.dot_general(
                ax_ref[:, r:r + 256], fwd_ref[...], (((0,), (0,)), ((), ())), preferred_element_type=f32)

        def butterfly(sign):
            def body(t, carry):
                r = pl.multiple_of(t * 16, 16)
                xs = [(z_s[pl.ds(n * S2 + r, 16), 0:256], z_s[pl.ds(n * S2 + r, 16), 256:512])
                      for n in range(R)]
                ys = _fft(xs, sign)
                for n in range(R):
                    b_s[pl.ds(n * S2 + r, 16), 0:256] = ys[n][0].astype(bf16)
                    b_s[pl.ds(n * S2 + r, 16), 256:512] = ys[n][1].astype(bf16)
                return carry
            jax.lax.fori_loop(0, S2 // 16, body, 0)

        butterfly(-1)
        for k1 in range(R):
            t = jnp.dot(ms_ref[k1], b_s[k1 * S2:(k1 + 1) * S2, :], preferred_element_type=f32)
            gr = t[0:256, 0:256] + t[256:512, 256:512]
            gi = t[0:256, 256:512] - t[256:512, 0:256]
            rows = pl.ds(k1, S2, stride=R)
            wr = jnp.concatenate([w_s[0, rows, :], w_s[1, rows, :]], axis=1)
            wi = jnp.concatenate([w_s[2, rows, :], w_s[3, rows, :]], axis=1)
            yr = (gr * wr - gi * wi).astype(bf16)
            yi = (gr * wi + gi * wr).astype(bf16)
            rhs = jnp.concatenate([jnp.concatenate([yr, yi], axis=1),
                                   jnp.concatenate([-yi, yr], axis=1)], axis=0)
            z_s[k1 * S2:(k1 + 1) * S2, :] = jax.lax.dot_general(
                ms_ref[k1], rhs, (((0,), (0,)), ((), ())), preferred_element_type=f32)
        butterfly(+1)
        for r in range(0, S, 256):
            y = jnp.dot(b_s[r:r + 256, :], inv_ref[...], preferred_element_type=f32)
            o_ref[0, r:r + 256, 0:M] = (y * (1.0 / (S * M))).astype(bf16)


@jax.jit
def pallas_concat_heads__spectral_gfnet__compressed_kv_cla__prompt_kernel(
    A_x, A_w_r, A_w_i, B_x, B_c_kv, B_w_q, B_w_uk, B_w_uv, B_w_o,
):
    def full(shape):
        n = len(shape)
        return pl.BlockSpec(shape, lambda h: (0,) * n, pipeline_mode=pl.Buffered(1))

    return pl.pallas_call(
        _kernel,
        grid=(H + 1,),
        in_specs=[
            full((M, S)), full((NF, S)), full((NF, S)),
            full(_FWD.shape), full(_INV.shape), full(_MS.shape),
            full((M, S)),
        ] + [pl.BlockSpec(memory_space=pltpu.MemorySpace.HBM)] * 5 + [
        ],
        out_specs=pl.BlockSpec((1, S, 2 * M), lambda h: (0, 0, 0)),
        out_shape=jax.ShapeDtypeStruct((1, S, 2 * M), jnp.bfloat16),
        scratch_shapes=[
            pltpu.VMEM((S, D), jnp.bfloat16), pltpu.VMEM((S, D), jnp.bfloat16),
            pltpu.VMEM((S, D), jnp.bfloat16), pltpu.VMEM((S, M), jnp.float32),
            pltpu.VMEM((S, 512), jnp.float32), pltpu.VMEM((S, 512), jnp.bfloat16),
            pltpu.VMEM((4, S, 128), jnp.float32), pltpu.VMEM((S, M), jnp.bfloat16),
            pltpu.VMEM((S, DC), jnp.bfloat16),
            pltpu.VMEM((M, H, D), jnp.bfloat16), pltpu.VMEM((DC, H, D), jnp.bfloat16),
            pltpu.VMEM((DC, H, D), jnp.bfloat16),
            pltpu.VMEM((H, M, D), jnp.bfloat16), pltpu.VMEM((H, DC, D), jnp.bfloat16),
            pltpu.VMEM((H, DC, D), jnp.bfloat16), pltpu.VMEM((H, M, D), jnp.bfloat16),
            pltpu.SemaphoreType.DMA((5,)),
        ],
        compiler_params=pltpu.CompilerParams(
            dimension_semantics=("arbitrary",), vmem_limit_bytes=110 * 1024 * 1024),
    )(A_x[0].T, A_w_r.T, A_w_i.T, _FWD, _INV, _MS,
      B_x[0].T, B_c_kv[0], B_w_q, B_w_uk, B_w_uv, B_w_o.transpose(0, 2, 1))
```

```python
import functools
import math

import jax
import jax.numpy as jnp
import ml_dtypes
import numpy as np
import jax.experimental.pallas as pl
import jax.experimental.pallas.tpu as pltpu

S, M, H, D, DC = 2048, 448, 16, 256, 1024
MH = M // 2
NF = MH + 1
R = 16
S2 = S // R
BF = ml_dtypes.bfloat16
SCOPES = False
CFG = dict(tq=256, pchunk=512, emit=2, inter=1, axc=4, rc=16, rl=256, qc=256, qstatic=1, kc=2048, mid=0)


def _consts():
    dd = np.arange(MH, dtype=np.float64)[:, None]
    m = np.arange(128, dtype=np.float64)[None, :]
    fwd, inv = [], []
    for par, nb in ((0, MH // 2 + 1), (1, MH // 2)):
        k = 2 * m + par
        ang = 2 * np.pi * ((dd * k) % M) / M
        valid = m < nb
        c, s = np.cos(ang) * valid, np.sin(ang) * valid
        fwd.append(np.concatenate([c, -s], axis=1))
        wt = np.where((k == 0) | (k == MH), 1.0, 2.0)
        inv.append(np.concatenate([(c * wt).T, (-s * wt).T], axis=0))
    k2 = np.arange(S2)
    mf, mi = [], []
    for k1 in range(R):
        a = 2 * np.pi * (((k1 + R * k2)[:, None] * k2[None, :]) % S) / S
        mf.append(np.concatenate([np.cos(a), np.sin(a)], axis=0))
        mi.append(np.concatenate([np.cos(a).T, np.sin(a).T], axis=0))
    return (np.stack(fwd).astype(BF), np.stack(inv).astype(BF),
            np.stack(mf).astype(BF), np.stack(mi).astype(BF))


_FWD, _INV, _MF, _MI = _consts()


def _fft(xs, sign):
    n = len(xs)
    if n == 1:
        return xs
    ev, od = _fft(xs[0::2], sign), _fft(xs[1::2], sign)
    out = [None] * n
    h = n // 2
    for k in range(h):
        er, ei = ev[k]
        orr, oi = od[k]
        if k == 0:
            tr, ti = orr, oi
        elif 4 * k == n:
            if sign < 0:
                out[k] = (er + oi, ei - orr)
                out[k + h] = (er - oi, ei + orr)
            else:
                out[k] = (er - oi, ei + orr)
                out[k + h] = (er + oi, ei - orr)
            continue
        elif 8 * k == n or 8 * k == 3 * n:
            r = math.sqrt(0.5)
            a, b = orr + oi, orr - oi
            if 8 * k == n:
                tr, ti = (a, -b) if sign < 0 else (b, a)
            else:
                tr, ti = (-b, -a) if sign < 0 else (-a, b)
            sr = 1.0 if (tr is a or tr is b) else -1.0
            si = 1.0 if (ti is a or ti is b) else -1.0
            if 8 * k == n:
                pr, pi_ = (a, b) if sign < 0 else (b, a)
                cr, ci = (r, -r) if sign < 0 else (r, r)
            else:
                pr, pi_ = (b, a) if sign < 0 else (a, b)
                cr, ci = (-r, -r) if sign < 0 else (-r, r)
            del sr, si, tr, ti
            tr, ti = pr * cr, pi_ * ci
        else:
            c = math.cos(2 * math.pi * k / n)
            s = sign * math.sin(2 * math.pi * k / n)
            tr, ti = orr * c - oi * s, orr * s + oi * c
        out[k] = (er + tr, ei + ti)
        out[k + h] = (er - tr, ei - ti)
    return out


class _Scope:
    def __init__(self, name):
        self.cm = jax.named_scope(name) if SCOPES else None

    def __enter__(self):
        if self.cm is not None:
            self.cm.__enter__()

    def __exit__(self, *a):
        if self.cm is not None:
            self.cm.__exit__(*a)


def _kernel(ax_hbm, wr_hbm, wi_hbm, fwd_hbm, inv_hbm, mf_hbm, mi_hbm,
            xt_hbm, c_hbm, wq_hbm, wuk_hbm, wuv_hbm, wo_hbm,
            o_hbm,
            ax_s, wr_s, wi_s, fwd_s, inv_s, mf_s, mi_s,
            z_s, b_s, w_s,
            xt_s, c_s, rq_s, rk_s, rv_s, wq_s, wuk_s, wuv_s, wo_s,
            q_s, k_s, o_s, xs_s, vt_s, acct_s, s_buf, sems, osems):
    f32, bf16, i32 = jnp.float32, jnp.bfloat16, jnp.int32
    AXC = CFG["axc"]
    AW = S // AXC
    pairs = dict(fwd=(fwd_hbm, fwd_s), wr=(wr_hbm, wr_s), wi=(wi_hbm, wi_s),
                 mf=(mf_hbm, mf_s), mi=(mi_hbm, mi_s), inv=(inv_hbm, inv_s),
                 xt=(xt_hbm, xt_s), wq=(wq_hbm, rq_s),
                 c=(c_hbm, c_s), wuk=(wuk_hbm, rk_s), wuv=(wuv_hbm, rv_s), wo=(wo_hbm, wo_s))
    for j in range(AXC):
        pairs["ax%d" % j] = (ax_hbm.at[:, j * AW:(j + 1) * AW], ax_s.at[:, j * AW:(j + 1) * AW])
    cp = {n: pltpu.make_async_copy(a, b, sems.at[i]) for i, (n, (a, b)) in enumerate(pairs.items())}
    out_a = pltpu.make_async_copy(o_s.at[:, 0:384], o_hbm.at[0, :, 0:384], osems.at[0])
    TQ = CFG["tq"]
    NQ = S // TQ
    out_b = [pltpu.make_async_copy(o_s.at[i * TQ:(i + 1) * TQ, 384:896],
                                   o_hbm.at[0, i * TQ:(i + 1) * TQ, 384:896], osems.at[1 + i])
             for i in range(NQ)]
    tn = (((0,), (0,)), ((), ()))
    nt = (((1,), (1,)), ((), ()))

    def start(*names):
        for n in names:
            cp[n].start()

    def wait(*names):
        with _Scope("wait_" + names[0]):
            for n in names:
                cp[n].wait()

    def relayout_rows(src, dst, r, n):
        rc, rl = CFG["rc"], CFG["rl"]
        for t in range(0, n, rc):
            for l in range(0, D, rl):
                dst[:, pl.ds(r + t, rc), l:l + rl] = jnp.swapaxes(src[pl.ds(r + t, rc), :, l:l + rl], 0, 1)

    def relayout(src, dst, n):
        with _Scope("relayout"):
            def body(t, carry):
                relayout_rows(src, dst, pl.multiple_of(t * 64, 64), 64)
                return carry
            jax.lax.fori_loop(0, n // 64, body, 0)

    start("fwd", "ax0", "ax1")

    with _Scope("dft_d"):
        cp["fwd"].wait()
        for j in range(AXC):
            cp["ax%d" % j].wait()
            if j + 2 < AXC:
                start("ax%d" % (j + 2))
            elif j + 2 == AXC:
                start("mf", "wr")
            else:
                start("wi")
            for r in range(j * AW, (j + 1) * AW, 256):
                x1 = ax_s[0:MH, r:r + 256].astype(f32)
                x2 = ax_s[MH:M, r:r + 256].astype(f32)
                z_s[r:r + 256, 0:256] = jax.lax.dot_general(
                    (x1 + x2).astype(bf16), fwd_s[0], tn, preferred_element_type=f32)
                z_s[r:r + 256, 256:512] = jax.lax.dot_general(
                    (x1 - x2).astype(bf16), fwd_s[1], tn, preferred_element_type=f32)

    def butterfly(sign):
        def body(t, carry):
            r = pl.multiple_of(t * 16, 16)
            for l in (0, 256):
                xs = [(z_s[pl.ds(n * S2 + r, 16), l:l + 128], z_s[pl.ds(n * S2 + r, 16), l + 128:l + 256])
                      for n in range(R)]
                ys = _fft(xs, sign)
                for n in range(R):
                    b_s[pl.ds(n * S2 + r, 16), l:l + 128] = ys[n][0].astype(bf16)
                    b_s[pl.ds(n * S2 + r, 16), l + 128:l + 256] = ys[n][1].astype(bf16)
            return carry
        with _Scope("butterfly"):
            jax.lax.fori_loop(0, S2 // 16, body, 0)

    butterfly(-1)
    wait("wr", "wi", "mf")
    start("mi", "inv", "xt", "wq")
    with _Scope("wprep"):
        lane_ok = jax.lax.broadcasted_iota(i32, (16, 256), 0) < 1
        for j, w_ref in enumerate((wr_s, wi_s)):
            for r in range(0, S, 256):
                u = pltpu.bitcast(w_ref[0:MH, r:r + 256], i32)
                ev = pltpu.bitcast(u << 16, f32)
                od = pltpu.bitcast(u & jnp.int32(-65536), f32)
                last = jnp.broadcast_to(w_ref[MH:NF, r:r + 256].astype(f32), (16, 256))
                last = jnp.where(lane_ok, last, 0.0)
                ev = jnp.concatenate([ev, last], axis=0)
                od = jnp.concatenate([od, jnp.zeros((16, 256), f32)], axis=0)
                w_s[j, r:r + 256, :] = ev.T
                w_s[2 + j, r:r + 256, :] = od.T
    with _Scope("dft_s"):
        def fwd_k(k1):
            r0 = k1 * S2 if isinstance(k1, int) else pl.multiple_of(k1 * S2, S2)
            t = jnp.dot(mf_s[k1], b_s[pl.ds(r0, S2), :], preferred_element_type=f32)
            rows = pl.ds(k1, S2, stride=R)
            for p, l in enumerate((0, 256)):
                gr = t[0:128, l:l + 128] + t[128:256, l + 128:l + 256]
                gi = t[0:128, l + 128:l + 256] - t[128:256, l:l + 128]
                wr = w_s[2 * p, rows, :]
                wi = w_s[2 * p + 1, rows, :]
                b_s[pl.ds(r0, S2), l:l + 128] = (gr * wr - gi * wi).astype(bf16)
                b_s[pl.ds(r0, S2), l + 128:l + 256] = (gr * wi + gi * wr).astype(bf16)

        def inv_k(k1):
            r0 = k1 * S2 if isinstance(k1, int) else pl.multiple_of(k1 * S2, S2)
            t = jnp.dot(mi_s[k1], b_s[pl.ds(r0, S2), :], preferred_element_type=f32)
            for l in (0, 256):
                z_s[pl.ds(r0, S2), l:l + 128] = t[0:128, l:l + 128] - t[128:256, l + 128:l + 256]
                z_s[pl.ds(r0, S2), l + 128:l + 256] = t[0:128, l + 128:l + 256] + t[128:256, l:l + 128]

        if CFG["mid"] == 0:
            for k1 in range(R):
                fwd_k(k1)
            cp["mi"].wait()
            for k1 in range(R):
                inv_k(k1)
        elif CFG["mid"] == 1:
            cp["mi"].wait()
            for k1 in range(R + 1):
                if k1 < R:
                    fwd_k(k1)
                if k1 > 0:
                    inv_k(k1 - 1)
        else:
            U = CFG["mid"]
            def fb(g, carry):
                for u in range(U):
                    fwd_k(g * U + u)
                return carry
            def ib(g, carry):
                for u in range(U):
                    inv_k(g * U + u)
                return carry
            jax.lax.fori_loop(0, R // U, fb, 0)
            cp["mi"].wait()
            jax.lax.fori_loop(0, R // U, ib, 0)
    butterfly(+1)
    wait("inv")
    start("wuk")
    with _Scope("idft_d"):
        sc = 1.0 / (S * M)
        for r in range(0, S, 256):
            e = jnp.dot(b_s[r:r + 256, 0:256], inv_s[0], preferred_element_type=f32)
            o = jnp.dot(b_s[r:r + 256, 256:512], inv_s[1], preferred_element_type=f32)
            y1 = (e + o) * sc
            y2 = (e - o) * sc
            o_s[r:r + 256, 0:MH] = y1.astype(bf16)
            o_s[r:r + 256, MH:384] = y2[:, 0:160].astype(bf16)
            y2t = jnp.concatenate([y2[:, 160:MH], jnp.zeros((256, 64), f32)], axis=1)
            acct_s[0:64, r:r + 256] = y2t.T[0:64]
    out_a.start()

    wait("xt", "wq")
    start("wuv", "c")
    relayout(rq_s, wq_s, M)
    with _Scope("xpose"):
        for r in range(0, S, 256):
            xs_s[r:r + 256, :] = xt_s[:, r:r + 256].astype(f32).T.astype(bf16)
    qscale = (D ** -0.5) * math.log2(math.e)

    def qloop(lo, hi, src=None, dst=None):
        def qbody(h, carry):
            qc = CFG["qc"]
            for n, r in enumerate(range(0, S, qc)):
                q = jnp.dot(xs_s[r:r + qc, :], wq_s[h], preferred_element_type=f32)
                q_s[h, r:r + qc, :] = (q * qscale).astype(bf16)
                if src is not None:
                    per = DC // (hi - lo)
                    sub = per * qc // S
                    relayout_rows(src, dst, (h - lo) * per + n * sub if CFG["qstatic"] else pl.multiple_of((h - lo) * per + n * sub, 16), sub)
            return carry
        with _Scope("q_all"):
            if src is not None and CFG["qstatic"]:
                for hh in range(lo, hi):
                    qbody(hh, 0)
            else:
                jax.lax.fori_loop(lo, hi, qbody, 0)

    if CFG["inter"]:
        qloop(0, 6)
        wait("wuk")
        start("wo")
        qloop(6, 10, rk_s, wuk_s)
        wait("wuv")
        qloop(10, 14, rv_s, wuv_s)
        qloop(14, 16)
    else:
        qloop(0, 16)
        start("wo")
        wait("wuk")
        relayout(rk_s, wuk_s, DC)
        wait("wuv")
        relayout(rv_s, wuv_s, DC)
    wait("c", "wo")

    def emit_block(i, new=None):
        cols = slice(i * TQ, (i + 1) * TQ)
        if new is None:
            blk = acct_s[:, cols]
        else:
            blk = jnp.concatenate([acct_s[0:64, cols], new], axis=0)
        o_s[cols, 384:896] = blk.T.astype(bf16)

    def head_c(h, carry, emit):
        PC = CFG["pchunk"]
        KC = CFG["kc"]
        W = 256
        NB = S // W
        tt = (((0,), (1,)), ((), ()))
        sbuf = [s_buf.at[j] for j in range(2)]

        def kproj(r, n):
            k_s[r:r + n, :] = jnp.dot(c_s[r:r + n, :], wuk_s[h], preferred_element_type=f32).astype(bf16)

        def vproj(r, n):
            vt_s[:, r:r + n] = jax.lax.dot_general(wuv_s[h], c_s[r:r + n, :], tt,
                                                   preferred_element_type=f32).astype(bf16)
        row = jax.lax.broadcasted_iota(i32, (128, 128), 0)
        col = jax.lax.broadcasted_iota(i32, (128, 128), 1)
        tri = row <= col

        def chunks(L):
            out, a = [], 0
            while a < L - 128:
                n = min(KC, L - 128 - a)
                out.append((a, n))
                a += n
            out.append((L - 128, 128))
            return out

        def colmax(x):
            return jnp.max(x.reshape(x.shape[0] // 8, 8, x.shape[1]), axis=0)

        def colsum(x):
            return jnp.sum(x.reshape(x.shape[0] // 8, 8, x.shape[1]), axis=0)

        def s_chunk(i, a, n, m8):
            r0 = i * W
            b = sbuf[i % 2]
            q = q_s[h, r0:r0 + W, :]
            st = jax.lax.dot_general(k_s[a:a + n, :], q, nt, preferred_element_type=f32)
            if a == r0:
                st = jnp.concatenate([jnp.where(tri, st[:, 0:128], -1e30), st[:, 128:256]], axis=1)
                se = jax.lax.dot_general(k_s[a + 128:a + 256, :], q[128:256], nt, preferred_element_type=f32)
                se = jnp.where(tri, se, -1e30)
                b[a + 128:a + 256, 128:256] = se
                me = colmax(se)
                ms = colmax(st)
                ms = jnp.concatenate([ms[:, 0:128], jnp.maximum(ms[:, 128:256], me)], axis=1)
            else:
                ms = colmax(st)
            b[a:a + n, :] = st
            return ms if m8 is None else jnp.maximum(m8, ms)

        def fin_chunk(i, a, n, m, state):
            r0 = i * W
            b = sbuf[i % 2]
            l8, ctx = state
            p = jnp.exp2(b[a:a + n, :] - m)
            ls = colsum(p)
            c = jnp.dot(vt_s[:, a:a + n], p.astype(bf16), preferred_element_type=f32)
            if a == r0:
                pe = jnp.exp2(b[a + 128:a + 256, 128:256] - m[:, 128:256])
                ls = jnp.concatenate([ls[:, 0:128], ls[:, 128:256] + colsum(pe)], axis=1)
                ce = jnp.dot(vt_s[:, a + 128:a + 256], pe.astype(bf16), preferred_element_type=f32)
                c = jnp.concatenate([c[:, 0:128], c[:, 128:256] + ce], axis=1)
            l8 = ls if l8 is None else l8 + ls
            ctx = c if ctx is None else ctx + c
            return l8, ctx

        def outproj(i, state):
            l8, ctx = state
            l = jnp.sum(l8, axis=0, keepdims=True)
            ctx = (ctx * (1.0 / l)).astype(bf16)
            new = acct_s[64:512, i * W:(i + 1) * W] + jnp.dot(wo_s[h], ctx, preferred_element_type=f32)
            acct_s[64:512, i * W:(i + 1) * W] = new
            if emit:
                emit_block(i, new)
                if isinstance(h, int):
                    out_b[i].start()
                else:
                    pl.when(h == H - 1)(out_b[i].start)

        for r in range(0, S, PC):
            kproj(r, PC)
            vproj(r, PC)
        m8 = None
        for (a, n) in chunks(128):
            m8 = s_chunk(0, a, n, m8)
        pend = None
        for i in range(NB):
            m = jnp.max(m8, axis=0, keepdims=True)
            fc = chunks(i * W + 128)
            sc = chunks((i + 1) * W + 128) if i + 1 < NB else []
            state = (None, None)
            m8 = None
            order = []
            for j in range(max(len(fc), len(sc))):
                if j < len(sc):
                    order.append(("s", sc[j]))
                if j < len(fc):
                    order.append(("f", fc[j]))
                if j == 0 and pend is not None:
                    order.append(("o", None))
            for kind, arg in order:
                if kind == "s":
                    m8 = s_chunk(i + 1, arg[0], arg[1], m8)
                elif kind == "f":
                    state = fin_chunk(i, arg[0], arg[1], m, state)
                else:
                    outproj(*pend)
                    pend = None
            pend = (i, state)
        outproj(*pend)
        return carry

    acct_s[64:512, :] = jnp.zeros((M, S), f32)
    with _Scope("heads"):
        if CFG["emit"] == 2:
            jax.lax.fori_loop(0, H - 1, functools.partial(head_c, emit=False), 0)
            head_c(H - 1, 0, emit=True)
        else:
            jax.lax.fori_loop(0, H, functools.partial(head_c, emit=bool(CFG["emit"])), 0)
    if not CFG["emit"]:
        with _Scope("emit"):
            for i in range(NQ):
                emit_block(i)
                out_b[i].start()
    out_a.wait()
    for c_ in out_b:
        c_.wait()


@jax.jit
def pallas_concat_heads__spectral_gfnet__compressed_kv_cla__prompt_kernel(
    A_x, A_w_r, A_w_i, B_x, B_c_kv, B_w_q, B_w_uk, B_w_uv, B_w_o,
):
    bf16, f32 = jnp.bfloat16, jnp.float32
    hbm = pl.BlockSpec(memory_space=pltpu.MemorySpace.HBM)
    return pl.pallas_call(
        _kernel,
        in_specs=[hbm] * 13,
        out_specs=hbm,
        out_shape=jax.ShapeDtypeStruct((1, S, 2 * M), bf16),
        scratch_shapes=[
            pltpu.VMEM((M, S), bf16), pltpu.VMEM((NF, S), bf16), pltpu.VMEM((NF, S), bf16),
            pltpu.VMEM(_FWD.shape, bf16), pltpu.VMEM(_INV.shape, bf16),
            pltpu.VMEM(_MF.shape, bf16), pltpu.VMEM(_MI.shape, bf16),
            pltpu.VMEM((S, 512), f32), pltpu.VMEM((S, 512), bf16), pltpu.VMEM((4, S, 128), f32),
            pltpu.VMEM((M, S), bf16), pltpu.VMEM((S, DC), bf16),
            pltpu.VMEM((M, H, D), bf16), pltpu.VMEM((DC, H, D), bf16), pltpu.VMEM((DC, H, D), bf16),
            pltpu.VMEM((H, M, D), bf16), pltpu.VMEM((H, DC, D), bf16), pltpu.VMEM((H, DC, D), bf16),
            pltpu.VMEM((H, M, D), bf16),
            pltpu.VMEM((H, S, D), bf16), pltpu.VMEM((S, D), bf16),
            pltpu.VMEM((S, 2 * M), bf16), pltpu.VMEM((S, M), bf16),
            pltpu.VMEM((D, S), bf16), pltpu.VMEM((512, S), f32), pltpu.VMEM((2, S, 256), f32),
            pltpu.SemaphoreType.DMA((12 + CFG["axc"],)), pltpu.SemaphoreType.DMA((1 + S // CFG["tq"],)),
        ],
        compiler_params=pltpu.CompilerParams(vmem_limit_bytes=110 * 1024 * 1024, flags=CFG.get("flags")),
    )(A_x[0].T, A_w_r.T, A_w_i.T, _FWD, _INV, _MF, _MI,
      B_x[0].T, B_c_kv[0], B_w_q, B_w_uk, B_w_uv, B_w_o.transpose(0, 2, 1))
```

```python
import functools
import math

import jax
import jax.numpy as jnp
import ml_dtypes
import numpy as np
import jax.experimental.pallas as pl
import jax.experimental.pallas.tpu as pltpu

S, M, H, D, DC = 2048, 448, 16, 256, 1024
MH = M // 2
NF = MH + 1
R = 16
S2 = S // R
BF = ml_dtypes.bfloat16
SCOPES = False
CFG = dict(tq=256, pchunk=1024, emit=2, inter=1, axc=4, rc=16, rl=256, qc=256, qstatic=1, kc=2048, mid=0, loops=1, loops2=0, g1=(), la=2, p2=('mf',), p3=('wr', 'wi'), pb=('mi', 'inv', 'xt', 'wq'))


def _consts():
    dd = np.arange(MH, dtype=np.float64)[:, None]
    m = np.arange(128, dtype=np.float64)[None, :]
    fwd, inv = [], []
    for par, nb in ((0, MH // 2 + 1), (1, MH // 2)):
        k = 2 * m + par
        ang = 2 * np.pi * ((dd * k) % M) / M
        valid = m < nb
        c, s = np.cos(ang) * valid, np.sin(ang) * valid
        fwd.append(np.concatenate([c, -s], axis=1))
        wt = np.where((k == 0) | (k == MH), 1.0, 2.0)
        inv.append(np.concatenate([(c * wt).T, (-s * wt).T], axis=0))
    k2 = np.arange(S2)
    mf, mi = [], []
    for k1 in range(R):
        a = 2 * np.pi * (((k1 + R * k2)[:, None] * k2[None, :]) % S) / S
        mf.append(np.concatenate([np.cos(a), np.sin(a)], axis=0))
        mi.append(np.concatenate([np.cos(a).T, np.sin(a).T], axis=0))
    return (np.stack(fwd).astype(BF), np.stack(inv).astype(BF),
            np.stack(mf).astype(BF), np.stack(mi).astype(BF))


_FWD, _INV, _MF, _MI = _consts()


def _fft(xs, sign):
    n = len(xs)
    if n == 1:
        return xs
    ev, od = _fft(xs[0::2], sign), _fft(xs[1::2], sign)
    out = [None] * n
    h = n // 2
    for k in range(h):
        er, ei = ev[k]
        orr, oi = od[k]
        if k == 0:
            tr, ti = orr, oi
        elif 4 * k == n:
            if sign < 0:
                out[k] = (er + oi, ei - orr)
                out[k + h] = (er - oi, ei + orr)
            else:
                out[k] = (er - oi, ei + orr)
                out[k + h] = (er + oi, ei - orr)
            continue
        elif 8 * k == n or 8 * k == 3 * n:
            r = math.sqrt(0.5)
            a, b = orr + oi, orr - oi
            if 8 * k == n:
                pr, pi_ = (a, b) if sign < 0 else (b, a)
                cr, ci = (r, -r) if sign < 0 else (r, r)
            else:
                pr, pi_ = (b, a) if sign < 0 else (a, b)
                cr, ci = (-r, -r) if sign < 0 else (-r, r)
            tr, ti = pr * cr, pi_ * ci
        else:
            c = math.cos(2 * math.pi * k / n)
            s = sign * math.sin(2 * math.pi * k / n)
            tr, ti = orr * c - oi * s, orr * s + oi * c
        out[k] = (er + tr, ei + ti)
        out[k + h] = (er - tr, ei - ti)
    return out


class _Scope:
    def __init__(self, name):
        self.cm = jax.named_scope(name) if SCOPES else None

    def __enter__(self):
        if self.cm is not None:
            self.cm.__enter__()

    def __exit__(self, *a):
        if self.cm is not None:
            self.cm.__exit__(*a)


def _kernel(ax_hbm, wr_hbm, wi_hbm, fwd_hbm, inv_hbm, mf_hbm, mi_hbm,
            xt_hbm, c_hbm, wq_hbm, wuk_hbm, wuv_hbm, wo_hbm,
            o_hbm,
            ax_s, wr_s, wi_s, fwd_s, inv_s, mf_s, mi_s,
            z_s, b_s, w_s,
            xt_s, c_s, rq_s, rk_s, rv_s, wq_s, wuk_s, wuv_s, wo_s,
            q_s, k_s, o_s, xs_s, vt_s, acct_s, s_buf, ca_s, sems, osems, axsems):
    f32, bf16, i32 = jnp.float32, jnp.bfloat16, jnp.int32
    AXC = CFG["axc"]
    AW = S // AXC
    pairs = dict(fwd=(fwd_hbm, fwd_s), wr=(wr_hbm, wr_s), wi=(wi_hbm, wi_s),
                 mf=(mf_hbm, mf_s), mi=(mi_hbm, mi_s), inv=(inv_hbm, inv_s),
                 xt=(xt_hbm, xt_s), wq=(wq_hbm, rq_s),
                 c=(c_hbm, c_s), wuk=(wuk_hbm, rk_s), wuv=(wuv_hbm, rv_s), wo=(wo_hbm, wo_s))
    cp = {n: pltpu.make_async_copy(a, b, sems.at[i]) for i, (n, (a, b)) in enumerate(pairs.items())}
    out_a = pltpu.make_async_copy(o_s.at[:, 0:384], o_hbm.at[0, :, 0:384], osems.at[0])
    TQ = CFG["tq"]
    NQ = S // TQ
    out_b = [pltpu.make_async_copy(o_s.at[i * TQ:(i + 1) * TQ, 384:896],
                                   o_hbm.at[0, i * TQ:(i + 1) * TQ, 384:896], osems.at[1 + i])
             for i in range(NQ)]
    tn = (((0,), (0,)), ((), ()))
    nt = (((1,), (1,)), ((), ()))

    def start(*names):
        for n in names:
            cp[n].start()

    def wait(*names):
        with _Scope("wait_" + names[0]):
            for n in names:
                cp[n].wait()

    def relayout_rows(src, dst, r, n):
        rc, rl = CFG["rc"], CFG["rl"]
        for t in range(0, n, rc):
            for l in range(0, D, rl):
                dst[:, pl.ds(r + t, rc), l:l + rl] = jnp.swapaxes(src[pl.ds(r + t, rc), :, l:l + rl], 0, 1)

    def relayout_st(src, dst, r, n):
        for t in range(0, n, 16):
            x1 = jnp.swapaxes(src[pl.ds(r + t, 16)], 0, 1)
            x2 = jnp.swapaxes(src[pl.ds(DC // 2 + r + t, 16)], 0, 1)
            b11, b12 = x1[:, :, 0:128], x1[:, :, 128:256]
            b21, b22 = x2[:, :, 0:128], x2[:, :, 128:256]
            f11, f12, f21, f22 = (b.astype(f32) for b in (b11, b12, b21, b22))
            ops = ((f11 + f22).astype(bf16), b11, (f12 - f22).astype(bf16), (f21 - f11).astype(bf16),
                   b22, (f11 + f12).astype(bf16), (f21 + f22).astype(bf16))
            for i, o in enumerate(ops):
                dst[:, i, pl.ds(r + t, 16), :] = o

    def relayout(src, dst, n):
        with _Scope("relayout"):
            def body(t, carry):
                relayout_rows(src, dst, pl.multiple_of(t * 64, 64), 64)
                return carry
            jax.lax.fori_loop(0, n // 64, body, 0)

    def ax_copy(j):
        cols = pl.ds(j * AW, AW) if isinstance(j, int) else pl.ds(pl.multiple_of(j * AW, AW), AW)
        return pltpu.make_async_copy(ax_hbm.at[:, cols], ax_s.at[:, cols], axsems.at[j])

    start("fwd")
    LA = CFG["la"]
    for j in range(LA):
        ax_copy(j).start()
    start(*CFG["g1"])

    def dft_d(j, carry):
        ax_copy(j).wait()
        if isinstance(j, int):
            if j + LA < AXC:
                ax_copy(j + LA).start()
        else:
            pl.when(j + LA < AXC)(lambda: ax_copy(jnp.minimum(j + LA, AXC - 1)).start())
        if isinstance(j, int):
            start(*CFG.get("p%d" % j, ()))
        else:
            for jj in range(AXC):
                if CFG.get("p%d" % jj):
                    pl.when(j == jj)(functools.partial(start, *CFG["p%d" % jj]))
        for r0 in range(0, AW, 256):
            r = j * AW + r0
            r = r if isinstance(r, int) else pl.multiple_of(r, 256)
            x1 = ax_s[0:MH, pl.ds(r, 256)].astype(f32)
            x2 = ax_s[MH:M, pl.ds(r, 256)].astype(f32)
            z_s[pl.ds(r, 256), 0:256] = jax.lax.dot_general(
                (x1 + x2).astype(bf16), fwd_s[0], tn, preferred_element_type=f32)
            z_s[pl.ds(r, 256), 256:512] = jax.lax.dot_general(
                (x1 - x2).astype(bf16), fwd_s[1], tn, preferred_element_type=f32)
        return carry

    def loop(n, body):
        if CFG["loops"]:
            jax.lax.fori_loop(0, n, body, 0)
        else:
            for j in range(n):
                body(j, 0)

    def loop2(n, body):
        if CFG["loops2"]:
            jax.lax.fori_loop(0, n, body, 0)
        else:
            for j in range(n):
                body(j, 0)

    with _Scope("dft_d"):
        cp["fwd"].wait()
        loop(AXC, dft_d)

    def butterfly(sign):
        def body(t, carry):
            r = pl.multiple_of(t * 16, 16)
            for l in (0, 256):
                xs = [(z_s[pl.ds(n * S2 + r, 16), l:l + 128], z_s[pl.ds(n * S2 + r, 16), l + 128:l + 256])
                      for n in range(R)]
                ys = _fft(xs, sign)
                for n in range(R):
                    b_s[pl.ds(n * S2 + r, 16), l:l + 128] = ys[n][0].astype(bf16)
                    b_s[pl.ds(n * S2 + r, 16), l + 128:l + 256] = ys[n][1].astype(bf16)
            return carry
        with _Scope("butterfly"):
            jax.lax.fori_loop(0, S2 // 16, body, 0)

    start(*CFG.get("pd", ()))
    butterfly(-1)
    start(*CFG.get("pb", ()))
    def fwd_k(k1):
        rows = slice(k1 * S2, (k1 + 1) * S2)
        t = jnp.dot(mf_s[k1], b_s[rows, :], preferred_element_type=f32)
        for l in (0, 256):
            z_s[rows, l:l + 128] = t[0:128, l:l + 128] + t[128:256, l + 128:l + 256]
            z_s[rows, l + 128:l + 256] = t[0:128, l + 128:l + 256] - t[128:256, l:l + 128]

    def inv_k(k1):
        rows = slice(k1 * S2, (k1 + 1) * S2)
        srows = pl.ds(k1, S2, stride=R)
        ys = []
        for p, l in enumerate((0, 256)):
            gr, gi = z_s[rows, l:l + 128], z_s[rows, l + 128:l + 256]
            wr, wi = w_s[2 * p, srows, :], w_s[2 * p + 1, srows, :]
            ys += [(gr * wr - gi * wi).astype(bf16), (gr * wi + gi * wr).astype(bf16)]
        t = jnp.dot(mi_s[k1], jnp.concatenate(ys, axis=1), preferred_element_type=f32)
        for l in (0, 256):
            z_s[rows, l:l + 128] = t[0:128, l:l + 128] - t[128:256, l + 128:l + 256]
            z_s[rows, l + 128:l + 256] = t[0:128, l + 128:l + 256] + t[128:256, l:l + 128]

    wait("mf")
    with _Scope("dft_s1"):
        for k1 in range(R):
            fwd_k(k1)
    start(*CFG.get("ps", ()))
    wait("wr", "wi")
    with _Scope("wprep"):
        lane_ok = jax.lax.broadcasted_iota(i32, (16, 256), 0) < 1
        def wprep(t, carry):
            r = t * 256 if isinstance(t, int) else pl.multiple_of(t * 256, 256)
            for j, w_ref in enumerate((wr_s, wi_s)):
                u = pltpu.bitcast(w_ref[0:MH, pl.ds(r, 256)], i32)
                ev = pltpu.bitcast(u << 16, f32)
                od = pltpu.bitcast(u & jnp.int32(-65536), f32)
                last = jnp.broadcast_to(w_ref[MH:NF, pl.ds(r, 256)].astype(f32), (16, 256))
                last = jnp.where(lane_ok, last, 0.0)
                ev = jnp.concatenate([ev, last], axis=0)
                od = jnp.concatenate([od, jnp.zeros((16, 256), f32)], axis=0)
                w_s[j, pl.ds(r, 256), :] = ev.T
                w_s[2 + j, pl.ds(r, 256), :] = od.T
            return carry
        loop2(S // 256, wprep)
    wait("mi")
    with _Scope("dft_s2"):
        for k1 in range(R):
            inv_k(k1)
    butterfly(+1)
    wait("inv")
    start("wuk")
    with _Scope("idft_d"):
        sc = 1.0 / (S * M)
        def idft(t, carry):
            r = t * 256 if isinstance(t, int) else pl.multiple_of(t * 256, 256)
            rows = pl.ds(r, 256)
            e = jnp.dot(b_s[rows, 0:256], inv_s[0], preferred_element_type=f32)
            o = jnp.dot(b_s[rows, 256:512], inv_s[1], preferred_element_type=f32)
            y1 = (e + o) * sc
            y2 = (e - o) * sc
            o_s[rows, 0:MH] = y1.astype(bf16)
            o_s[rows, MH:384] = y2[:, 0:160].astype(bf16)
            y2t = jnp.concatenate([y2[:, 160:MH], jnp.zeros((256, 64), f32)], axis=1)
            acct_s[0:64, rows] = y2t.T[0:64]
            return carry
        loop2(S // 256, idft)
    out_a.start()

    wait("xt", "wq")
    start("wuv", "c")
    relayout(rq_s, wq_s, M)
    HS, HC = S // 2, DC // 2

    def wcomb(x, y, sgn):
        x, y = x.astype(f32), y.astype(f32)
        return (x + y if sgn > 0 else x - y).astype(bf16)

    def strassen7(a, b11, b12, b21, b22):
        w = (lambda: wcomb(b11, b22, 1), lambda: b11, lambda: wcomb(b12, b22, -1), lambda: wcomb(b21, b11, -1),
             lambda: b22, lambda: wcomb(b11, b12, 1), lambda: wcomb(b21, b22, 1))
        m = [jnp.dot(a[i], w[i](), preferred_element_type=f32) for i in range(7)]
        return (m[0] + m[3] - m[4] + m[6], m[2] + m[4], m[1] + m[3], m[0] - m[1] + m[2] + m[5])

    with _Scope("xpose"):
        for t in range(0, HS, 256):
            a11, a12 = xt_s[0:MH, t:t + 256].astype(f32), xt_s[MH:M, t:t + 256].astype(f32)
            a21 = xt_s[0:MH, HS + t:HS + t + 256].astype(f32)
            a22 = xt_s[MH:M, HS + t:HS + t + 256].astype(f32)
            for i, o in enumerate((a11 + a22, a21 + a22, a11, a22, a11 + a12, a21 - a11, a12 - a22)):
                xs_s[i, t:t + 256, :] = o.T.astype(bf16)
    qscale = (D ** -0.5) * math.log2(math.e)

    def acomb(r):
        a11, a12 = c_s[r:r + 128, 0:HC].astype(f32), c_s[r:r + 128, HC:DC].astype(f32)
        a21, a22 = c_s[HS + r:HS + r + 128, 0:HC].astype(f32), c_s[HS + r:HS + r + 128, HC:DC].astype(f32)
        for i, o in enumerate((a11 + a22, a21 + a22, a11 + a12, a21 - a11, a12 - a22)):
            ca_s[i, r:r + 128, :] = o.astype(bf16)

    def qloop(lo, hi, src=None, dst=None, ac=False):
        def qbody(h, carry):
            qc = CFG["qc"]
            for n, r in enumerate(range(0, HS, qc)):
                w = wq_s.at[h]
                quads = strassen7([xs_s[i, r:r + qc, :] for i in range(7)],
                                  w[0:MH, 0:128], w[0:MH, 128:256], w[MH:M, 0:128], w[MH:M, 128:256])
                for qd, (ro, lo_) in zip(quads, ((0, 0), (0, 128), (HS, 0), (HS, 128))):
                    q_s[h, ro + r:ro + r + qc, lo_:lo_ + 128] = (qd * qscale).astype(bf16)
                if src is not None:
                    per = DC // (hi - lo)
                    sub = per * qc // HS
                    relayout_rows(src, dst, (h - lo) * per + n * sub, sub)
                if ac:
                    acomb(((h - lo) * (HS // qc) + n) * 128)
            return carry
        with _Scope("q_all"):
            if (src is not None or ac) and CFG["qstatic"]:
                for hh in range(lo, hi):
                    qbody(hh, 0)
            else:
                jax.lax.fori_loop(lo, hi, qbody, 0)

    if CFG["inter"]:
        qloop(0, 6)
        wait("wuk")
        start("wo")
        qloop(6, 10, rk_s, wuk_s)
        wait("wuv")
        qloop(10, 14, rv_s, wuv_s)
        wait("c", "wo")
        qloop(14, 16, ac=True)
    else:
        qloop(0, 16)
        start("wo")
        wait("wuk")
        relayout(rk_s, wuk_s, DC)
        wait("wuv")
        relayout(rv_s, wuv_s, DC)
    def strassen(w7, r, n):
        a = (ca_s[0, r:r + n, :], ca_s[1, r:r + n, :], c_s[r:r + n, 0:HC], c_s[HS + r:HS + r + n, HC:DC],
             ca_s[2, r:r + n, :], ca_s[3, r:r + n, :], ca_s[4, r:r + n, :])
        return strassen7(a, w7[0:HC, 0:128], w7[0:HC, 128:256], w7[HC:DC, 0:128], w7[HC:DC, 128:256])

    def emit_block(i, new=None):
        cols = slice(i * TQ, (i + 1) * TQ)
        if new is None:
            blk = acct_s[:, cols]
        else:
            blk = jnp.concatenate([acct_s[0:64, cols], new], axis=0)
        o_s[cols, 384:896] = blk.T.astype(bf16)

    def head_c(h, carry, emit):
        PC = CFG["pchunk"]
        KC = CFG["kc"]
        W = 256
        NB = S // W
        tt = (((0,), (1,)), ((), ()))
        sbuf = [s_buf.at[j] for j in range(2)]

        def kproj(r, n):
            k_s[r:r + n, :] = jnp.dot(c_s[r:r + n, :], wuk_s[h], preferred_element_type=f32).astype(bf16)

        def vproj(r, n):
            vt_s[:, r:r + n] = jax.lax.dot_general(wuv_s[h], c_s[r:r + n, :], tt,
                                                   preferred_element_type=f32).astype(bf16)
        row = jax.lax.broadcasted_iota(i32, (128, 128), 0)
        col = jax.lax.broadcasted_iota(i32, (128, 128), 1)
        tri = row <= col

        def chunks(L):
            out, a = [], 0
            while a < L - 128:
                n = min(KC, L - 128 - a)
                out.append((a, n))
                a += n
            out.append((L - 128, 128))
            return out

        def colmax(x):
            return jnp.max(x.reshape(x.shape[0] // 8, 8, x.shape[1]), axis=0)

        def colsum(x):
            return jnp.sum(x.reshape(x.shape[0] // 8, 8, x.shape[1]), axis=0)

        def s_chunk(i, a, n, m8):
            r0 = i * W
            b = sbuf[i % 2]
            q = q_s[h, r0:r0 + W, :]
            st = jax.lax.dot_general(k_s[a:a + n, :], q, nt, preferred_element_type=f32)
            if a == r0:
                st = jnp.concatenate([jnp.where(tri, st[:, 0:128], -1e30), st[:, 128:256]], axis=1)
                se = jax.lax.dot_general(k_s[a + 128:a + 256, :], q[128:256], nt, preferred_element_type=f32)
                se = jnp.where(tri, se, -1e30)
                b[a + 128:a + 256, 128:256] = se
                me = colmax(se)
                ms = colmax(st)
                ms = jnp.concatenate([ms[:, 0:128], jnp.maximum(ms[:, 128:256], me)], axis=1)
            else:
                ms = colmax(st)
            b[a:a + n, :] = st
            return ms if m8 is None else jnp.maximum(m8, ms)

        def fin_chunk(i, a, n, m, state):
            r0 = i * W
            b = sbuf[i % 2]
            l8, ctx = state
            p = jnp.exp2(b[a:a + n, :] - m)
            ls = colsum(p)
            c = jnp.dot(vt_s[:, a:a + n], p.astype(bf16), preferred_element_type=f32)
            if a == r0:
                pe = jnp.exp2(b[a + 128:a + 256, 128:256] - m[:, 128:256])
                ls = jnp.concatenate([ls[:, 0:128], ls[:, 128:256] + colsum(pe)], axis=1)
                ce = jnp.dot(vt_s[:, a + 128:a + 256], pe.astype(bf16), preferred_element_type=f32)
                c = jnp.concatenate([c[:, 0:128], c[:, 128:256] + ce], axis=1)
            l8 = ls if l8 is None else l8 + ls
            ctx = c if ctx is None else ctx + c
            return l8, ctx

        def outproj(i, state):
            l8, ctx = state
            l = jnp.sum(l8, axis=0, keepdims=True)
            ctx = (ctx * (1.0 / l)).astype(bf16)
            old = acct_s[64:512, i * W:(i + 1) * W]
            if not isinstance(h, int):
                old = jnp.where(h > 0, old, 0.0)
            new = old + jnp.dot(wo_s[h], ctx, preferred_element_type=f32)
            acct_s[64:512, i * W:(i + 1) * W] = new
            if emit:
                emit_block(i, new)
                if isinstance(h, int):
                    out_b[i].start()
                else:
                    pl.when(h == H - 1)(out_b[i].start)

        for r in range(0, HS, PC):
            c11, c12, c21, c22 = strassen(wuk_s.at[h], r, PC)
            k_s[r:r + PC, 0:128] = c11.astype(bf16)
            k_s[r:r + PC, 128:256] = c12.astype(bf16)
            k_s[HS + r:HS + r + PC, 0:128] = c21.astype(bf16)
            k_s[HS + r:HS + r + PC, 128:256] = c22.astype(bf16)
            c11, c12, c21, c22 = strassen(wuv_s.at[h], r, PC)
            vt_s[0:128, r:r + PC] = c11.T.astype(bf16)
            vt_s[128:256, r:r + PC] = c12.T.astype(bf16)
            vt_s[0:128, HS + r:HS + r + PC] = c21.T.astype(bf16)
            vt_s[128:256, HS + r:HS + r + PC] = c22.T.astype(bf16)
        m8 = None
        for (a, n) in chunks(128):
            m8 = s_chunk(0, a, n, m8)
        pend = None
        for i in range(NB):
            m = jnp.max(m8, axis=0, keepdims=True)
            fc = chunks(i * W + 128)
            sc = chunks((i + 1) * W + 128) if i + 1 < NB else []
            state = (None, None)
            m8 = None
            order = []
            for j in range(max(len(fc), len(sc))):
                if j < len(sc):
                    order.append(("s", sc[j]))
                if j < len(fc):
                    order.append(("f", fc[j]))
                if j == 0 and pend is not None:
                    order.append(("o", None))
            for kind, arg in order:
                if kind == "s":
                    m8 = s_chunk(i + 1, arg[0], arg[1], m8)
                elif kind == "f":
                    state = fin_chunk(i, arg[0], arg[1], m, state)
                else:
                    outproj(*pend)
                    pend = None
            pend = (i, state)
        outproj(*pend)
        return carry

    with _Scope("heads"):
        if CFG["emit"] == 2:
            jax.lax.fori_loop(0, H - 1, functools.partial(head_c, emit=False), 0)
            head_c(H - 1, 0, emit=True)
        else:
            jax.lax.fori_loop(0, H, functools.partial(head_c, emit=bool(CFG["emit"])), 0)
    if not CFG["emit"]:
        with _Scope("emit"):
            for i in range(NQ):
                emit_block(i)
                out_b[i].start()
    out_a.wait()
    for c_ in out_b:
        c_.wait()


@jax.jit
def pallas_concat_heads__spectral_gfnet__compressed_kv_cla__prompt_kernel(
    A_x, A_w_r, A_w_i, B_x, B_c_kv, B_w_q, B_w_uk, B_w_uv, B_w_o,
):
    bf16, f32 = jnp.bfloat16, jnp.float32
    hbm = pl.BlockSpec(memory_space=pltpu.MemorySpace.HBM)
    return pl.pallas_call(
        _kernel,
        in_specs=[hbm] * 13,
        out_specs=hbm,
        out_shape=jax.ShapeDtypeStruct((1, S, 2 * M), bf16),
        scratch_shapes=[
            pltpu.VMEM((M, S), bf16), pltpu.VMEM((NF, S), bf16), pltpu.VMEM((NF, S), bf16),
            pltpu.VMEM(_FWD.shape, bf16), pltpu.VMEM(_INV.shape, bf16),
            pltpu.VMEM(_MF.shape, bf16), pltpu.VMEM(_MI.shape, bf16),
            pltpu.VMEM((S, 512), f32), pltpu.VMEM((S, 512), bf16), pltpu.VMEM((4, S, 128), f32),
            pltpu.VMEM((M, S), bf16), pltpu.VMEM((S, DC), bf16),
            pltpu.VMEM((M, H, D), bf16), pltpu.VMEM((DC, H, D), bf16), pltpu.VMEM((DC, H, D), bf16),
            pltpu.VMEM((H, M, D), bf16), pltpu.VMEM((H, DC, D), bf16), pltpu.VMEM((H, DC, D), bf16),
            pltpu.VMEM((H, M, D), bf16),
            pltpu.VMEM((H, S, D), bf16), pltpu.VMEM((S, D), bf16),
            pltpu.VMEM((S, 2 * M), bf16), pltpu.VMEM((7, S // 2, MH), bf16),
            pltpu.VMEM((D, S), bf16), pltpu.VMEM((512, S), f32), pltpu.VMEM((2, S, 256), f32), pltpu.VMEM((5, S // 2, DC // 2), bf16),
            pltpu.SemaphoreType.DMA((12,)), pltpu.SemaphoreType.DMA((1 + S // CFG["tq"],)),
            pltpu.SemaphoreType.DMA((CFG["axc"],)),
        ],
        compiler_params=pltpu.CompilerParams(vmem_limit_bytes=116 * 1024 * 1024, flags=CFG.get("flags")),
    )(A_x[0].T, A_w_r.T, A_w_i.T, _FWD, _INV, _MF, _MI,
      B_x[0].T, B_c_kv[0], B_w_q, B_w_uk, B_w_uv, B_w_o.transpose(0, 2, 1))
```
